```python
import os as _os
_os.environ.setdefault('JAX_PLATFORMS', 'cpu')
import jax
import jax.numpy as jnp

def _softmax(x, axis=-1):
    return jax.nn.softmax(x, axis=axis)

def _gelu(x):
    return jax.nn.gelu(x, approximate=True)

def _silu(x):
    return jax.nn.silu(x)

def _sigmoid(x):
    return jax.nn.sigmoid(x)

def _layernorm(x, axis=-1, eps=1e-05):
    m = jnp.mean(x, axis=axis, keepdims=True)
    v = jnp.var(x, axis=axis, keepdims=True)
    return (x - m) / jnp.sqrt(v + eps)

def _scatter_add(tgt, idx, src, axis=0):
    return tgt.at[idx].add(src)

def _segment_sum(src, seg, n):
    return jax.ops.segment_sum(src, seg, n)

class _Rng:

    def __init__(self, key):
        self._k = key

    def _next(self):
        self._k, sub = jax.random.split(self._k)
        return sub

    def normal(self, shape):
        return jax.random.normal(self._next(), shape, dtype=jnp.bfloat16)

    def randint(self, lo, hi, shape):
        return jax.random.randint(self._next(), shape, lo, hi, dtype=jnp.int32)

    def uniform(self, shape, lo=0.0, hi=1.0):
        return jax.random.uniform(self._next(), shape, jnp.bfloat16, lo, hi)

    def permutation(self, n):
        return jax.random.permutation(self._next(), n)
kernel_name = 'standalone__conformer_family_e_branchformer__speech'

def setup_inputs():
    _rng = _Rng(jax.random.key(int.from_bytes(__import__("os").urandom(4), "little")))
    _w = lambda a: (lambda t: t.astype(jnp.bfloat16) if jnp.issubdtype(t.dtype, jnp.floating) else t)(jnp.asarray(a))
    B, T, D, K = (2, 4000, 512, 5)
    return {'x': _w((lambda *s: _rng.normal(s) * 0.05)(B, T, D)), 'w_qkv': _w((lambda *s: _rng.normal(s) * 0.05)(D, 3 * D)), 'w_att_out': _w((lambda *s: _rng.normal(s) * 0.05)(D, D)), 'w_mlp_in': _w((lambda *s: _rng.normal(s) * 0.05)(D, 2 * D)), 'dw_csgu': _w((lambda *s: _rng.normal(s) * 0.05)(K, D)), 'w_mlp_out': _w((lambda *s: _rng.normal(s) * 0.05)(D, D)), 'dw_merge': _w((lambda *s: _rng.normal(s) * 0.05)(K, 2 * D)), 'w_merge': _w((lambda *s: _rng.normal(s) * 0.05)(2 * D, D))}

def reference(x, w_qkv, w_att_out, w_mlp_in, dw_csgu, w_mlp_out, dw_merge, w_merge):
    B, T, D = x.shape
    K = dw_csgu.shape[0]
    pad = K // 2
    xa = _layernorm(x, axis=-1)
    qkv = jnp.einsum('btd,de->bte', xa, w_qkv)
    q, k, v = (qkv[..., :D].copy(), qkv[..., D:2 * D].copy(), qkv[..., 2 * D:].copy())
    scores = jnp.einsum('btd,bsd->bts', q, k) * D ** (-0.5)
    p = _softmax(scores, axis=-1)
    attn = jnp.einsum('bts,bsd->btd', p, v)
    glob = jnp.einsum('btd,de->bte', attn, w_att_out)
    xc = _layernorm(x, axis=-1)
    h = _gelu(jnp.einsum('btd,de->bte', xc, w_mlp_in))
    u, g = (h[..., :D].copy(), h[..., D:].copy())
    g = _layernorm(g, axis=-1)
    gp = jnp.pad(g, ((0, 0), (pad, pad), (0, 0)))
    gc = jnp.zeros_like(g)
    for i in range(K):
        gc = gc + gp[:, i:i + T, :] * dw_csgu[i][None, None, :]
    loc = jnp.einsum('btd,de->bte', u * gc, w_mlp_out)
    m = jnp.concatenate([glob, loc], axis=-1)
    mp = jnp.pad(m, ((0, 0), (pad, pad), (0, 0)))
    mc = jnp.zeros_like(m)
    for i in range(K):
        mc = mc + mp[:, i:i + T, :] * dw_merge[i][None, None, :]
    m = m + mc
    return x + jnp.einsum('btc,cd->btd', m, w_merge)
```

```python
import math
import jax
import jax.numpy as jnp
from jax import lax
from jax.experimental import pallas as pl
from jax.experimental.pallas import tpu as pltpu

NEG = -1e30
NT = (((1,), (1,)), ((), ()))
EPS = 1e-5
HALO = 8
LANE = 128
RC = 80
RL = 16


def _fold(x, op):
    n = x.shape[1] // LANE
    r = x[:, 0:LANE]
    for j in range(1, n):
        r = op(r, x[:, j * LANE:(j + 1) * LANE])
    return r


def _ln(x):
    d = x.shape[-1]
    mu = jnp.sum(x, axis=-1, keepdims=True) * (1.0 / d)
    xc = x - mu
    var = jnp.sum(xc * xc, axis=-1, keepdims=True) * (1.0 / d)
    return xc * lax.rsqrt(var + EPS)


def _gelu(x):
    c = math.sqrt(2.0 / math.pi)
    inner = x * (c + (c * 0.044715) * (x * x))
    hx = 0.5 * x
    return hx + hx * jnp.tanh(inner)


class _NullScope:
    def __enter__(self):
        return self

    def __exit__(self, *a):
        return False


@jax.jit
def pallas_standalone__conformer_family_e_branchformer__speech_kernel(
        x, w_qkv, w_att_out, w_mlp_in, dw_csgu, w_mlp_out, dw_merge, w_merge):
    TQ, TK, ostarts, ub = 400, 512, (3, 6, 8, 9), 1
    scope = lambda name: _NullScope()
    B, T, D = x.shape
    K = dw_csgu.shape[0]
    pad = K // 2
    TP = -(-T // TK) * TK
    NQ = T // TQ
    NC = TP // TK
    ND = D // LANE
    NKT = TK // LANE
    qscale = (D ** -0.5) * math.log2(math.e)
    f32, bf16, i32 = jnp.float32, jnp.bfloat16, jnp.int32

    def kernel(x_hbm, wqkv_hbm, wo_hbm, win_hbm, dwc_hbm, wout_hbm, dwm_hbm, wm_hbm, o_hbm,
               x_s, wqkv_s, wo_s, win_s, wout_s, wm_s, dwc_in, dwm_in,
               wqk_s, wvo_s, dwc_s, dwm_s, one_s,
               xa_s, q_s, v_s, u_s, g_s, m_s, z_s, mm_s, s_s, mrun, mfin, l_s, acc_s,
               w_sems, x_sems):
        def rows(i, off=0, n=TQ, al=16):
            if isinstance(i, int):
                return pl.ds(i * TQ + off, n)
            return pl.ds(pl.multiple_of(i * TQ + off, al), n)

        def cat(ref, r, j0=0, j1=None):
            j1 = ref.shape[0] if j1 is None else j1
            return jnp.concatenate([ref[j, r, :] for j in range(j0, j1)], axis=1)

        def col(j):
            return slice(j * LANE, (j + 1) * LANE)

        def x_copy(b, i):
            return pltpu.make_async_copy(x_hbm.at[b, rows(i), :], x_s.at[b, rows(i), :],
                                         x_sems.at[b * NQ + i])

        def out_copy(b, i):
            return pltpu.make_async_copy(x_s.at[b, rows(i), :], o_hbm.at[b, rows(i), :],
                                         x_sems.at[b * NQ + i])

        c_qk = pltpu.make_async_copy(wqkv_hbm.at[:, pl.ds(0, 2 * D)], wqkv_s.at[:, pl.ds(0, 2 * D)], w_sems.at[0])
        c_v = pltpu.make_async_copy(wqkv_hbm.at[:, pl.ds(2 * D, D)], wqkv_s.at[:, pl.ds(2 * D, D)], w_sems.at[1])
        c_wo = pltpu.make_async_copy(wo_hbm, wo_s, w_sems.at[2])
        c_win = pltpu.make_async_copy(win_hbm, win_s, w_sems.at[3])
        c_dwc = pltpu.make_async_copy(dwc_hbm, dwc_in, w_sems.at[4])
        c_wout = pltpu.make_async_copy(wout_hbm, wout_s, w_sems.at[5])
        c_dwm = pltpu.make_async_copy(dwm_hbm, dwm_in, w_sems.at[6])
        c_wm = pltpu.make_async_copy(wm_hbm, wm_s, w_sems.at[7])

        c_qk.start()
        c_v.start()
        c_wo.start()
        x_copy(0, 0).start()
        c_win.start()
        x_copy(0, 1).start()
        x_copy(0, 2).start()
        one_s[...] = jnp.ones((8, LANE), i32)
        for j in range(ND):
            xa_s[j, T:TP, :] = jnp.zeros((TP - T, LANE), bf16)
            v_s[j, T:TP, :] = jnp.zeros((TP - T, LANE), bf16)
            g_s[j, 0:HALO, :] = jnp.zeros((HALO, LANE), f32)
            g_s[j, HALO + T:HALO + T + HALO, :] = jnp.zeros((HALO, LANE), f32)
        for j in range(2 * ND):
            m_s[j, 0:HALO, :] = jnp.zeros((HALO, LANE), f32)
            m_s[j, HALO + T:HALO + T + HALO, :] = jnp.zeros((HALO, LANE), f32)

        def tie(val, tok):
            if tok is None:
                return val
            true1 = one_s[0:1, :] != 0
            if val.dtype != f32:
                tok = lax.bitcast_convert_type(tok, val.dtype)
            if val.shape[1] != LANE:
                n = val.shape[1] // LANE
                return jnp.concatenate(
                    [jnp.where(true1, val[:, col(j)], tok) for j in range(n)], axis=1)
            return jnp.where(true1, val, tok)

        def conv_chunk(ref, w_ref, j, base, tok):
            acc = None
            for k in range(K):
                wk_ = tie(w_ref[k:k + 1, col(j)], tok)
                t = ref[j, pl.ds(base + k, RC), :] * wk_
                acc = t if acc is None else acc + t
            return acc

        def toks_from(res, n):
            pts = []
            for y in res:
                for t in range(y.shape[1] // LANE):
                    for tr in range(0, y.shape[0], 8):
                        pts.append((y, t, tr))
            out = []
            for k in range(n):
                y, t, tr = pts[(k * len(pts)) // n]
                out.append(y[tr:tr + 1, col(t)])
            return out

        NZ = ND * (TQ // RC)
        NL = TQ // RL

        def lnx(b, i, toks):
            for c in range(NL):
                r = rows(i, c * RL, RL)
                xb = x_s[b, r, :]
                if toks is not None:
                    xb = pltpu.bitcast(tie(pltpu.bitcast(xb, i32), toks[c]), bf16)
                xa = _ln(xb.astype(f32)).astype(bf16)
                for j in range(ND):
                    xa_s[j, r, :] = xa[:, col(j)]

        with scope("W0"):
            c_qk.wait()
        c_dwc.start()
        c_wout.start()
        for i in range(3, NQ):
            x_copy(0, i).start()
        with scope("prep1"):
            wq = wqkv_s[:, 0:D]
            wk = wqkv_s[:, D:2 * D]
            wqk = (lax.dot_general(wq, wk, NT, preferred_element_type=f32) * qscale).astype(bf16)
            for j in range(ND):
                wqk_s[j] = wqk[:, col(j)]
        with scope("W1"):
            c_v.wait()
            c_wo.wait()
            x_copy(0, 0).wait()
        with scope("prep2"):
            wvo = jnp.dot(wqkv_s[:, 2 * D:3 * D], wo_s[...], preferred_element_type=f32)
            for j in range(ND):
                wvo_s[j] = wvo[:, col(j)].astype(bf16)
            lnx(0, 0, toks_from([wvo], NL))
        with scope("W2"):
            c_win.wait()

        def batch(b, _):
            @pl.when(b > 0)
            def _():
                c_dwc.start()
                c_wout.start()

            def lng(i, toks):
                for c in range(NL):
                    r = rows(i, HALO + c * RL, RL, 8)
                    g = jnp.concatenate([tie(g_s[j, r, :], toks[c]) for j in range(ND)], axis=1)
                    g = _ln(g)
                    for j in range(ND):
                        g_s[j, r, :] = g[:, col(j)]

            def proj(i):
                xa = cat(xa_s, rows(i))
                res = []
                for j in range(ND):
                    y = jnp.dot(xa, win_s[:, D + j * LANE:D + (j + 1) * LANE], preferred_element_type=f32)
                    g_s[j, rows(i, HALO, TQ, 8), :] = _gelu(y)
                    res.append(y)
                for j in range(ND):
                    y = jnp.dot(xa, win_s[:, col(j)], preferred_element_type=f32)
                    u_s[j, rows(i), :] = _gelu(y)
                    res.append(y)
                for j in range(ND):
                    y = jnp.dot(xa, wvo_s[j], preferred_element_type=f32)
                    v_s[j, rows(i), :] = y.astype(bf16)
                    res.append(y)
                for j in range(ND):
                    y = jnp.dot(xa, wqk_s[j], preferred_element_type=f32)
                    q_s[j, rows(i), :] = y.astype(bf16)
                    res.append(y)
                return res

            def zcalc(i, toks):
                n = 0
                for j in range(ND):
                    for r0 in range(0, TQ, RC):
                        gc = conv_chunk(g_s, dwc_s, j, i * TQ + (HALO - pad) + r0, toks[n])
                        n += 1
                        u = u_s[j, rows(i, r0, RC), :]
                        z_s[j, rows(i, r0, RC), :] = (u * gc).astype(bf16)

            def loc(i):
                z = cat(z_s, rows(i))
                res = []
                for j in range(ND):
                    y = jnp.dot(z, wout_s[:, col(j)], preferred_element_type=f32)
                    m_s[ND + j, rows(i, HALO, TQ, 8), :] = y
                    res.append(y)
                return res

            def qk(qi, c):
                q = cat(q_s, rows(qi))
                k = cat(xa_s, pl.ds(c * TK, TK))
                s = lax.dot_general(q, k, NT, preferred_element_type=f32)
                if (c + 1) * TK > T:
                    cc = lax.broadcasted_iota(i32, (TQ, TK), 1) + c * TK
                    s = jnp.where(cc < T, s, NEG)
                s_s[c] = s
                mx = _fold(s, jnp.maximum)
                if c == 0:
                    mrun[...] = mx
                else:
                    mrun[...] = jnp.maximum(mrun[...], mx)
                return s

            def fin1():
                m = jnp.max(mrun[...], axis=1, keepdims=True)
                mfin[...] = jnp.broadcast_to(m, (TQ, LANE))

            with scope("A"):
                x_copy(b, 1).wait()
                x_copy(b, 2).wait()
                for i in range(NQ):
                    if i == 1:
                        c_dwc.wait()
                        c_wout.wait()
                        for t in range(3, 5):
                            x_copy(b, t).wait()
                        dwc_s[...] = dwc_in[...].astype(f32)
                    if i == 4:
                        for t in range(5, NQ):
                            x_copy(b, t).wait()
                    res = proj(i)
                    if i >= 2:
                        loc(i - 2)
                    if i + 1 < NQ:
                        lnx(b, i + 1, toks_from(res[0:8], NL))
                    lng(i, toks_from(res[5:12], NL))
                    if i >= 1:
                        zcalc(i - 1, toks_from(res[8:16], NZ))
                r8 = loc(NQ - 2)
                res = [qk(0, c) for c in range(NC // 2)]
                zcalc(NQ - 1, toks_from(r8 + res[0:1], NZ))
                loc(NQ - 1)
                res = [qk(0, c) for c in range(NC // 2, NC)]
                fin1()

            @pl.when(b == 0)
            def _():
                c_dwm.start()
                c_wm.start()

            @pl.when(b + 1 < B)
            def _():
                for i in range(NQ):
                    x_copy(b + 1, i).start()

            def ex(c):
                m = mfin[...]
                mt = jnp.concatenate([m] * NKT, axis=1)
                p = jnp.exp2(s_s[c] - mt)
                ls = _fold(p, jnp.add)
                if c == 0:
                    l_s[...] = ls
                else:
                    l_s[...] += ls
                return p.astype(bf16)

            def pv(p, c):
                r = jnp.dot(p, cat(v_s, pl.ds(c * TK, TK)), preferred_element_type=f32)
                if c == 0:
                    acc_s[...] = r
                else:
                    acc_s[...] += r
                return r

            def fin2(qi):
                l = jnp.sum(l_s[...], axis=1, keepdims=True)
                o = acc_s[...] * (1.0 / l)
                for j in range(ND):
                    m_s[j, rows(qi, HALO, TQ, 8), :] = o[:, col(j)]

            def b_tile(qi):
                for c in range(NC):
                    p = ex(c)
                    qk(qi + 1, c)
                    pv(p, c)
                fin1()
                fin2(qi)

            def b_body(it, _):
                for u in range(ub):
                    b_tile(it * ub + u)
                return 0
            with scope("Bloop"):
                lax.fori_loop(0, (NQ - 1) // ub, b_body, 0)

            @pl.when(b == 0)
            def _():
                c_dwm.wait()
                c_wm.wait()
                row = lax.broadcasted_iota(i32, (K, 2 * D), 0)
                dwm_s[...] = dwm_in[...].astype(f32) + jnp.where(row == pad, 1.0, 0.0)

            @pl.when(b + 1 < B)
            def _():
                x_copy(b + 1, 0).wait()

            def mcalc(i, toks):
                n = 0
                for j in range(2 * ND):
                    for r0 in range(0, TQ, RC):
                        mm_s[(i % 2) * 2 * ND + j, r0:r0 + RC, :] = conv_chunk(
                            m_s, dwm_s, j, i * TQ + (HALO - pad) + r0, toks[n]).astype(bf16)
                        n += 1

            def merge(i):
                a = cat(mm_s, slice(None), (i % 2) * 2 * ND, (i % 2 + 1) * 2 * ND)
                res = []
                for n in range(ND):
                    y = jnp.dot(a, wm_s[:, col(n)], preferred_element_type=f32)
                    xr = x_s[b, rows(i), col(n)].astype(f32)
                    x_s[b, rows(i), col(n)] = (xr + y).astype(bf16)
                    res.append(y)
                return res

            with scope("D"):
                res = []
                for c in range(NC):
                    res.append(pv(ex(c), c))
                mcalc(0, toks_from(res[1:], 2 * NZ))
                lnx(jnp.minimum(b + 1, B - 1), 0, toks_from(res[1:], NL))
                fin2(NQ - 1)
                for i in range(NQ):
                    res = merge(i)
                    if i + 1 < NQ:
                        mcalc(i + 1, toks_from(res, 2 * NZ))
                    if i in ostarts:
                        prev = [o for o in ostarts if o < i]
                        lo = prev[-1] + 1 if prev else 0
                        for t in range(lo, i + 1):
                            out_copy(b, t).start()
            return 0

        lax.fori_loop(0, B, batch, 0)
        with scope("Fin"):
            for b in range(B):
                for i in range(NQ):
                    out_copy(b, i).wait()

    any_spec = pl.BlockSpec(memory_space=pl.ANY)
    return pl.pallas_call(
        kernel,
        out_shape=jax.ShapeDtypeStruct((B, T, D), x.dtype),
        in_specs=[any_spec] * 8,
        out_specs=any_spec,
        scratch_shapes=[
            pltpu.VMEM((B, T, D), bf16),
            pltpu.VMEM((D, 3 * D), bf16),
            pltpu.VMEM((D, D), bf16),
            pltpu.VMEM((D, 2 * D), bf16),
            pltpu.VMEM((D, D), bf16),
            pltpu.VMEM((2 * D, D), bf16),
            pltpu.VMEM((K, D), bf16),
            pltpu.VMEM((K, 2 * D), bf16),
            pltpu.VMEM((ND, D, LANE), bf16),
            pltpu.VMEM((ND, D, LANE), bf16),
            pltpu.VMEM((K, D), f32),
            pltpu.VMEM((K, 2 * D), f32),
            pltpu.VMEM((8, LANE), i32),
            pltpu.VMEM((ND, TP, LANE), bf16),
            pltpu.VMEM((ND, T, LANE), bf16),
            pltpu.VMEM((ND, TP, LANE), bf16),
            pltpu.VMEM((ND, T, LANE), f32),
            pltpu.VMEM((ND, T + 2 * HALO, LANE), f32),
            pltpu.VMEM((2 * ND, T + 2 * HALO, LANE), f32),
            pltpu.VMEM((ND, T, LANE), bf16),
            pltpu.VMEM((4 * ND, TQ, LANE), bf16),
            pltpu.VMEM((NC, TQ, TK), f32),
            pltpu.VMEM((TQ, LANE), f32),
            pltpu.VMEM((TQ, LANE), f32),
            pltpu.VMEM((TQ, LANE), f32),
            pltpu.VMEM((TQ, D), f32),
            pltpu.SemaphoreType.DMA((8,)),
            pltpu.SemaphoreType.DMA((B * NQ,)),
        ],
        compiler_params=pltpu.CompilerParams(vmem_limit_bytes=120 * 1024 * 1024),
    )(x, w_qkv, w_att_out, w_mlp_in, dw_csgu, w_mlp_out, dw_merge, w_merge)
```

```python
import math

import jax
import jax.numpy as jnp
from jax import lax
from jax.experimental import pallas as pl
from jax.experimental.pallas import tpu as pltpu

NT = (((1,), (1,)), ((), ()))
EPS = 1e-5
LANE = 128
HALO = 8
TQ = 400
TK = 512
RC = 80
RL = 16
RE = 40
RR = 8


def _fold(x, op):
    r = x[:, 0:LANE]
    for j in range(1, x.shape[1] // LANE):
        r = op(r, x[:, j * LANE:(j + 1) * LANE])
    return r


def _ln(x):
    d = x.shape[-1]
    mu = jnp.sum(x, axis=-1, keepdims=True) * (1.0 / d)
    xc = x - mu
    var = jnp.sum(xc * xc, axis=-1, keepdims=True) * (1.0 / d)
    return xc * lax.rsqrt(var + EPS)


def _gelu(x):
    c = math.sqrt(2.0 / math.pi)
    inner = x * (c + (c * 0.044715) * (x * x))
    hx = 0.5 * x
    return hx + hx * jnp.tanh(inner)


@jax.jit
def pallas_standalone__conformer_family_e_branchformer__speech_kernel(
        x, w_qkv, w_att_out, w_mlp_in, dw_csgu, w_mlp_out, dw_merge, w_merge):
    B, T, D = x.shape
    K = dw_csgu.shape[0]
    pad = K // 2
    NQ = T // TQ
    NC = -(-T // TK)
    TP = NC * TK
    ND = D // LANE
    NKT = TK // LANE
    KF = (T // LANE) * LANE
    REM = T - KF
    LASTW = KF - (NC - 1) * TK
    QP = TQ + (-TQ) % LANE
    assert T % TQ == 0 and NQ >= 5 and D % LANE == 0 and pad <= HALO
    assert 0 < REM and REM % 16 == 0 and 0 < LASTW
    RPOS = 1
    corder = list(range(NC - 1))
    corder.insert(RPOS, NC - 1)
    out_starts = (3, 6, NQ - 2)
    qscale = (D ** -0.5) * math.log2(math.e)
    f32, bf16, i32 = jnp.float32, jnp.bfloat16, jnp.int32
    NZ = ND * (TQ // RC)
    NL = TQ // RL
    NE = TQ // RE

    def kernel(x_hbm, wqkv_hbm, wo_hbm, win_hbm, dwc_hbm, wout_hbm, dwm_hbm, wm_hbm, o_hbm,
               x_s, wqkv_s, wo_s, win_s, wout_s, wm_s, dwc_in, dwm_in,
               wqk_s, wvo_s, dwc_s, dwm_s, one_s,
               xa_s, q_s, v_s, u_s, g_s, m_s, z_s, mm_s, s_s, mrun, mfin, l_s, acc_s,
               prem_s, vrem_s, orem_s,
               w_sems, x_sems):
        def rows(i, off=0, n=TQ, al=16):
            if isinstance(i, int):
                return pl.ds(i * TQ + off, n)
            return pl.ds(pl.multiple_of(i * TQ + off, al), n)

        def cat(ref, r, j0=0, j1=None):
            j1 = ref.shape[0] if j1 is None else j1
            return jnp.concatenate([ref[j, r, :] for j in range(j0, j1)], axis=1)

        def col(j):
            return slice(j * LANE, (j + 1) * LANE)

        def x_copy(b, i):
            return pltpu.make_async_copy(x_hbm.at[b, rows(i), :], x_s.at[b, rows(i), :],
                                         x_sems.at[b * NQ + i])

        def out_copy(b, i):
            return pltpu.make_async_copy(x_s.at[b, rows(i), :], o_hbm.at[b, rows(i), :],
                                         x_sems.at[b * NQ + i])

        def out_col_copy(b, i, n):
            return pltpu.make_async_copy(x_s.at[b, rows(i), pl.ds(n * LANE, LANE)],
                                         o_hbm.at[b, rows(i), pl.ds(n * LANE, LANE)],
                                         w_sems.at[9 + n])

        c_qk = pltpu.make_async_copy(wqkv_hbm.at[:, pl.ds(0, 2 * D)],
                                     wqkv_s.at[:, pl.ds(0, 2 * D)], w_sems.at[0])
        c_v = pltpu.make_async_copy(wqkv_hbm.at[:, pl.ds(2 * D, D)],
                                    wqkv_s.at[:, pl.ds(2 * D, D)], w_sems.at[1])
        c_wo = pltpu.make_async_copy(wo_hbm, wo_s, w_sems.at[2])
        c_wing = pltpu.make_async_copy(win_hbm.at[:, pl.ds(D, D)],
                                       win_s.at[:, pl.ds(D, D)], w_sems.at[3])
        c_winu = pltpu.make_async_copy(win_hbm.at[:, pl.ds(0, D)],
                                       win_s.at[:, pl.ds(0, D)], w_sems.at[8])
        c_dwc = pltpu.make_async_copy(dwc_hbm, dwc_in, w_sems.at[4])
        c_wout = pltpu.make_async_copy(wout_hbm, wout_s, w_sems.at[5])
        c_dwm = pltpu.make_async_copy(dwm_hbm, dwm_in, w_sems.at[6])
        c_wm = pltpu.make_async_copy(wm_hbm, wm_s, w_sems.at[7])

        def ordered_start(cps):
            def body(i, c):
                for k, cp in enumerate(cps):
                    pl.when(i == k)(cp.start)
                return c
            lax.fori_loop(0, len(cps), body, 0)

        def tie(val, tok):
            if tok is None:
                return val
            true1 = one_s[0:1, :] != 0
            if val.dtype != f32:
                tok = lax.bitcast_convert_type(tok, val.dtype)
            if val.shape[1] != LANE:
                n = val.shape[1] // LANE
                return jnp.concatenate(
                    [jnp.where(true1, val[:, col(j)], tok) for j in range(n)], axis=1)
            return jnp.where(true1, val, tok)

        def toks_from(res, n):
            pts = []
            for y in res:
                for t in range(y.shape[1] // LANE):
                    for tr in range(0, y.shape[0], 8):
                        pts.append((y, t, tr))
            out = []
            for k in range(n):
                y, t, tr = pts[(k * len(pts)) // n]
                out.append(y[tr:tr + 1, col(t)])
            return out

        def conv_chunk(ref, w_ref, j, base, tok):
            acc = None
            for k in range(K):
                wk_ = tie(w_ref[k:k + 1, col(j)], tok)
                t = ref[j, pl.ds(base + k, RC), :] * wk_
                acc = t if acc is None else acc + t
            return acc

        def lnx(b, i, toks):
            for c in range(NL):
                r = rows(i, c * RL, RL)
                xb = x_s[b, r, :]
                if toks is not None:
                    xb = pltpu.bitcast(tie(pltpu.bitcast(xb, i32), toks[c]), bf16)
                xa = _ln(xb.astype(f32)).astype(bf16)
                for j in range(ND):
                    xa_s[j, r, :] = xa[:, col(j)]

        def lng(i, toks):
            for c in range(NL):
                r = rows(i, HALO + c * RL, RL, 8)
                g = jnp.concatenate([tie(g_s[j, r, :], toks[c]) for j in range(ND)], axis=1)
                g = _ln(g)
                for j in range(ND):
                    g_s[j, r, :] = g[:, col(j)]

        def proj_g(i):
            xa = cat(xa_s, rows(i))
            res = []
            for j in range(ND):
                y = jnp.dot(xa, win_s[:, D + j * LANE:D + (j + 1) * LANE],
                            preferred_element_type=f32)
                g_s[j, rows(i, HALO, TQ, 8), :] = _gelu(y)
                res.append(y)
            return res

        def proj_u(i):
            xa = cat(xa_s, rows(i))
            res = []
            for j in range(ND):
                y = jnp.dot(xa, win_s[:, col(j)], preferred_element_type=f32)
                u_s[j, rows(i), :] = _gelu(y)
                res.append(y)
            return res

        def proj_v(i):
            xa = cat(xa_s, rows(i))
            res = []
            for j in range(ND):
                y = jnp.dot(xa, wvo_s[j], preferred_element_type=f32)
                v_s[j, rows(i), :] = y.astype(bf16)
                res.append(y)
            return res

        def proj_q(i):
            xa = cat(xa_s, rows(i))
            res = []
            for j in range(ND):
                y = jnp.dot(xa, wqk_s[j], preferred_element_type=f32)
                q_s[j, rows(i), :] = y.astype(bf16)
                res.append(y)
            return res

        def prep_qk():
            wqk = lax.dot_general(wqkv_s[:, 0:D], wqkv_s[:, D:2 * D], NT,
                                  preferred_element_type=f32)
            for j in range(ND):
                wqk_s[j] = (wqk[:, col(j)] * qscale).astype(bf16)
            return wqk

        def prep_vo():
            wvo = jnp.dot(wqkv_s[:, 2 * D:3 * D], wo_s[...], preferred_element_type=f32)
            for j in range(ND):
                wvo_s[j] = wvo[:, col(j)].astype(bf16)

        def zcalc(i, toks):
            n = 0
            for j in range(ND):
                for r0 in range(0, TQ, RC):
                    gc = conv_chunk(g_s, dwc_s, j, i * TQ + (HALO - pad) + r0, toks[n])
                    n += 1
                    u = u_s[j, rows(i, r0, RC), :]
                    z_s[j, rows(i, r0, RC), :] = (u * gc).astype(bf16)

        def loc(i):
            z = cat(z_s, rows(i))
            res = []
            for j in range(ND):
                y = jnp.dot(z, wout_s[:, col(j)], preferred_element_type=f32)
                m_s[ND + j, rows(i, HALO, TQ, 8), :] = y
                res.append(y)
            return res

        def qk(qi, c):
            q = cat(q_s, rows(qi))
            if c == NC - 1:
                k = cat(xa_s, pl.ds(c * TK, LASTW))
                s0 = lax.dot_general(q, k, NT, preferred_element_type=f32)
                st = lax.dot_general(cat(xa_s, pl.ds(KF, REM)), cat(q_s, rows(qi, 0, QP)), NT,
                                     preferred_element_type=f32)
                st = jnp.concatenate([st, jnp.full((LANE - REM, QP), -jnp.inf, f32)], axis=0)
                s = jnp.concatenate([s0, st.T[:TQ, :]], axis=1)
            else:
                k = cat(xa_s, pl.ds(c * TK, TK))
                s = lax.dot_general(q, k, NT, preferred_element_type=f32)
            s_s[c] = s
            mx = _fold(s, jnp.maximum)
            if c == corder[0]:
                mrun[...] = mx
            else:
                mrun[...] = jnp.maximum(mrun[...], mx)
            return s

        def fin1():
            m = jnp.max(mrun[...], axis=1, keepdims=True)
            mfin[...] = jnp.broadcast_to(m, (TQ, LANE))

        def ex(c, toks):
            ps = []
            step = TQ if toks is None else RE
            for n, r0 in enumerate(range(0, TQ, step)):
                m = mfin[r0:r0 + step, :]
                if toks is not None:
                    m = tie(m, toks[n])
                mt = jnp.concatenate([m] * NKT, axis=1)
                p = jnp.exp2(s_s[c, r0:r0 + step, :] - mt)
                ls = _fold(p, jnp.add)
                if c == corder[0]:
                    l_s[r0:r0 + step, :] = ls
                else:
                    l_s[r0:r0 + step, :] += ls
                if c == NC - 1:
                    prem_s[r0:r0 + step, :] = p[:, LASTW:]
                    p = p[:, :LASTW]
                ps.append(p)
            return jnp.concatenate(ps, axis=0).astype(bf16)

        def pv(p, c):
            r = jnp.dot(p, cat(v_s, pl.ds(c * TK, p.shape[1])), preferred_element_type=f32)
            if c == corder[0]:
                acc_s[...] = r
            elif c != corder[-1]:
                acc_s[...] += r
            return r

        def pvrem(toks):
            for n, r0 in enumerate(range(0, TQ, RR)):
                pc = tie(prem_s[r0:r0 + RR, :], toks[n])
                accs = [None] * ND
                for k in range(REM):
                    pb = jnp.broadcast_to(pc[:, k:k + 1], (RR, LANE))
                    for j in range(ND):
                        t = pb * vrem_s[k:k + 1, col(j)]
                        accs[j] = t if accs[j] is None else accs[j] + t
                for j in range(ND):
                    orem_s[r0:r0 + RR, col(j)] = accs[j]

        def fin2(qi, r_last):
            l = jnp.sum(l_s[...], axis=1, keepdims=True)
            o = ((acc_s[...] + orem_s[...]) + r_last) * (1.0 / l)
            for j in range(ND):
                m_s[j, rows(qi, HALO, TQ, 8), :] = o[:, col(j)]

        def b_body(qi, carry):
            res = []
            prev = None
            for c in corder:
                p = ex(c, None if prev is None else toks_from(prev, NE))
                res.append(qk(qi + 1, c))
                r = pv(p, c)
                prev = [r[:, 0:D - LANE]]
            pvrem(toks_from(res[RPOS + 1:-1], TQ // RR))
            fin1()
            fin2(qi, r)
            return carry

        def mcalc(i, toks):
            n = 0
            for j in range(2 * ND):
                for r0 in range(0, TQ, RC):
                    mm_s[(i % 2) * 2 * ND + j, r0:r0 + RC, :] = conv_chunk(
                        m_s, dwm_s, j, i * TQ + (HALO - pad) + r0, toks[n]).astype(bf16)
                    n += 1

        def merge(b, i, stream_out):
            a = cat(mm_s, slice(None), (i % 2) * 2 * ND, (i % 2 + 1) * 2 * ND)
            res = []
            for n in range(ND):
                y = jnp.dot(a, wm_s[:, col(n)], preferred_element_type=f32)
                xr = x_s[b, rows(i), col(n)].astype(f32)
                x_s[b, rows(i), col(n)] = (xr + y).astype(bf16)
                if stream_out:
                    out_col_copy(b, i, n).start()
                res.append(y)
            return res

        ordered_start([x_copy(0, 0), c_wing, c_winu, c_qk, x_copy(0, 1), c_v, c_wo])
        one_s[...] = jnp.ones((8, LANE), i32)
        for j in range(ND):
            xa_s[j, T:TP, :] = jnp.zeros((TP - T, LANE), bf16)
            v_s[j, T:TP, :] = jnp.zeros((TP - T, LANE), bf16)
            q_s[j, T:T - TQ + QP, :] = jnp.zeros((QP - TQ, LANE), bf16)
            g_s[j, 0:HALO, :] = jnp.zeros((HALO, LANE), f32)
            g_s[j, HALO + T:HALO + T + HALO, :] = jnp.zeros((HALO, LANE), f32)
        for j in range(2 * ND):
            m_s[j, 0:HALO, :] = jnp.zeros((HALO, LANE), f32)
            m_s[j, HALO + T:HALO + T + HALO, :] = jnp.zeros((HALO, LANE), f32)
        ordered_start([x_copy(0, 2), c_dwc, c_wout] + [x_copy(0, i) for i in range(3, NQ)])

        x_copy(0, 0).wait()
        lnx(0, 0, None)
        c_wing.wait()
        proj_g(0)
        c_winu.wait()
        lng(0, toks_from(proj_u(0), NL))
        c_qk.wait()
        x_copy(0, 1).wait()
        rq = prep_qk()
        rq2 = proj_q(0)
        lnx(0, 1, toks_from([rq] + rq2[0:ND - 1], NL))
        c_v.wait()
        c_wo.wait()
        prep_vo()
        proj_v(0)

        for b in range(B):
            if b > 0:
                for i in range(1, NQ):
                    x_copy(b, i).wait()
            for i in range(1 if b == 0 else 0, NQ):
                if b == 0 and i == 1:
                    c_dwc.wait()
                    c_wout.wait()
                    for t in range(2, 5):
                        x_copy(0, t).wait()
                    dwc_s[...] = dwc_in[...].astype(f32)
                if b == 0 and i == 4:
                    for t in range(5, NQ):
                        x_copy(0, t).wait()
                res = proj_g(i) + proj_u(i) + proj_v(i) + proj_q(i)
                if i >= 2:
                    loc(i - 2)
                if i + 1 < NQ:
                    lnx(b, i + 1, toks_from(res[0:2 * ND], NL))
                lng(i, toks_from(res[ND + 1:3 * ND], NL))
                if i >= 1:
                    zcalc(i - 1, toks_from(res[2 * ND:4 * ND], NZ))
            r8 = loc(NQ - 2)
            res = [qk(0, c) for c in corder[:NC // 2]]
            zcalc(NQ - 1, toks_from(r8 + res[0:1], NZ))
            res = [qk(0, c) for c in corder[NC // 2:]]
            fin1()
            vrem_s[...] = cat(v_s, pl.ds(KF, REM)).astype(f32)
            if b == 0:
                c_dwm.start()
                c_wm.start()
            if b + 1 < B:
                for i in range(NQ):
                    x_copy(b + 1, i).start()

            lax.fori_loop(0, NQ - 1, b_body, 0)
            if b == 0:
                c_dwm.wait()
                row = lax.broadcasted_iota(i32, (K, 2 * D), 0)
                dwm_s[...] = dwm_in[...].astype(f32) + jnp.where(row == pad, 1.0, 0.0)

            res = []
            prev = loc(NQ - 1)[0:ND - 1]
            for c in corder:
                r = pv(ex(c, toks_from(prev, NE)), c)
                res.append(r)
                prev = [r[:, 0:D - LANE]]
            pvrem(toks_from(res[RPOS + 1:-1], TQ // RR))
            mcalc(0, toks_from(res[1:], 2 * NZ))
            fin2(NQ - 1, r)
            if b == 0:
                c_wm.wait()
            else:
                for i in range(NQ):
                    out_copy(b - 1, i).wait()
            if b + 1 < B:
                x_copy(b + 1, 0).wait()

            for i in range(NQ):
                res = merge(b, i, b == B - 1 and i == NQ - 1)
                if i + 1 < NQ:
                    mcalc(i + 1, toks_from(res, 2 * NZ))
                if i == NQ - 1 and b + 1 < B:
                    lnx(b + 1, 0, toks_from(res[0:ND - 1], NL))
                if b == B - 1 and i in out_starts:
                    done = [o for o in out_starts if o < i]
                    for t in range(done[-1] + 1 if done else 0, i + 1):
                        out_copy(b, t).start()
            if b < B - 1:
                for t in range(NQ):
                    out_copy(b, t).start()

        for i in range(NQ - 1):
            out_copy(B - 1, i).wait()
        for n in range(ND):
            out_col_copy(B - 1, NQ - 1, n).wait()

    any_spec = pl.BlockSpec(memory_space=pl.ANY)
    return pl.pallas_call(
        kernel,
        out_shape=jax.ShapeDtypeStruct((B, T, D), x.dtype),
        in_specs=[any_spec] * 8,
        out_specs=any_spec,
        scratch_shapes=[
            pltpu.VMEM((B, T, D), bf16),
            pltpu.VMEM((D, 3 * D), bf16),
            pltpu.VMEM((D, D), bf16),
            pltpu.VMEM((D, 2 * D), bf16),
            pltpu.VMEM((D, D), bf16),
            pltpu.VMEM((2 * D, D), bf16),
            pltpu.VMEM((K, D), bf16),
            pltpu.VMEM((K, 2 * D), bf16),
            pltpu.VMEM((ND, D, LANE), bf16),
            pltpu.VMEM((ND, D, LANE), bf16),
            pltpu.VMEM((K, D), f32),
            pltpu.VMEM((K, 2 * D), f32),
            pltpu.VMEM((8, LANE), i32),
            pltpu.VMEM((ND, TP, LANE), bf16),
            pltpu.VMEM((ND, T - TQ + QP, LANE), bf16),
            pltpu.VMEM((ND, TP, LANE), bf16),
            pltpu.VMEM((ND, T, LANE), f32),
            pltpu.VMEM((ND, T + 2 * HALO, LANE), f32),
            pltpu.VMEM((2 * ND, T + 2 * HALO, LANE), f32),
            pltpu.VMEM((ND, T, LANE), bf16),
            pltpu.VMEM((4 * ND, TQ, LANE), bf16),
            pltpu.VMEM((NC, TQ, TK), f32),
            pltpu.VMEM((TQ, LANE), f32),
            pltpu.VMEM((TQ, LANE), f32),
            pltpu.VMEM((TQ, LANE), f32),
            pltpu.VMEM((TQ, D), f32),
            pltpu.VMEM((TQ, LANE), f32),
            pltpu.VMEM((REM, D), f32),
            pltpu.VMEM((TQ, D), f32),
            pltpu.SemaphoreType.DMA((9 + ND,)),
            pltpu.SemaphoreType.DMA((B * NQ,)),
        ],
        compiler_params=pltpu.CompilerParams(vmem_limit_bytes=120 * 1024 * 1024),
    )(x, w_qkv, w_att_out, w_mlp_in, dw_csgu, w_mlp_out, dw_merge, w_merge)
```

```python
import math

import jax
import jax.numpy as jnp
from jax import lax
from jax.experimental import pallas as pl
from jax.experimental.pallas import tpu as pltpu

NT = (((1,), (1,)), ((), ()))
EPS = 1e-5
LANE = 128
HALO = 8
TQ = 400
TK = 512
RC = 80
RL = 16
RE = 40
RR = 8


def _fold(x, op):
    r = x[:, 0:LANE]
    for j in range(1, x.shape[1] // LANE):
        r = op(r, x[:, j * LANE:(j + 1) * LANE])
    return r


def _ln(x):
    d = x.shape[-1]
    mu = jnp.sum(x, axis=-1, keepdims=True) * (1.0 / d)
    xc = x - mu
    var = jnp.sum(xc * xc, axis=-1, keepdims=True) * (1.0 / d)
    return xc * lax.rsqrt(var + EPS)


def _gelu(x):
    c = math.sqrt(2.0 / math.pi)
    inner = x * (c + (c * 0.044715) * (x * x))
    hx = 0.5 * x
    return hx + hx * jnp.tanh(inner)


@jax.jit
def pallas_standalone__conformer_family_e_branchformer__speech_kernel(
        x, w_qkv, w_att_out, w_mlp_in, dw_csgu, w_mlp_out, dw_merge, w_merge):
    B, T, D = x.shape
    K = dw_csgu.shape[0]
    pad = K // 2
    NQ = T // TQ
    NC = -(-T // TK)
    TP = NC * TK
    ND = D // LANE
    NKT = TK // LANE
    KF = (T // LANE) * LANE
    REM = T - KF
    LASTW = KF - (NC - 1) * TK
    QP = TQ + (-TQ) % LANE
    assert T % TQ == 0 and NQ >= 5 and D % LANE == 0 and pad <= HALO
    assert 0 < REM and REM % 16 == 0 and 0 < LASTW
    RPOS = 1
    corder = list(range(NC - 1))
    corder.insert(RPOS, NC - 1)
    out_starts = (3, 6, NQ - 2)
    qscale = (D ** -0.5) * math.log2(math.e)
    f32, bf16, i32 = jnp.float32, jnp.bfloat16, jnp.int32
    NZ = ND * (TQ // RC)
    NL = TQ // RL
    NE = TQ // RE

    def kernel(x_hbm, wqkv_hbm, wo_hbm, win_hbm, dwc_hbm, wout_hbm, dwm_hbm, wm_hbm, o_hbm,
               x_s, wqkv_s, wo_s, win_s, wout_s, wm_s, dwc_in, dwm_in,
               wqk_s, wvo_s, dwc_s, dwm_s, one_s,
               xa_s, q_s, v_s, u_s, g_s, m_s, z_s, mm_s, s_s, mrun, mfin, l_s, acc_s,
               prem_s, vrem_s, orem_s,
               w_sems, x_sems):
        def rows(i, off=0, n=TQ, al=16):
            if isinstance(i, int):
                return pl.ds(i * TQ + off, n)
            return pl.ds(pl.multiple_of(i * TQ + off, al), n)

        def cat(ref, r, j0=0, j1=None):
            j1 = ref.shape[0] if j1 is None else j1
            return jnp.concatenate([ref[j, r, :] for j in range(j0, j1)], axis=1)

        def col(j):
            return slice(j * LANE, (j + 1) * LANE)

        def x_copy(b, i):
            return pltpu.make_async_copy(x_hbm.at[b, rows(i), :], x_s.at[b, rows(i), :],
                                         x_sems.at[b * NQ + i])

        def out_copy(b, i):
            return pltpu.make_async_copy(x_s.at[b, rows(i), :], o_hbm.at[b, rows(i), :],
                                         x_sems.at[b * NQ + i])

        def out_col_copy(b, i, n):
            return pltpu.make_async_copy(x_s.at[b, rows(i), pl.ds(n * LANE, LANE)],
                                         o_hbm.at[b, rows(i), pl.ds(n * LANE, LANE)],
                                         w_sems.at[9 + n])

        c_qk = pltpu.make_async_copy(wqkv_hbm.at[:, pl.ds(0, 2 * D)],
                                     wqkv_s.at[:, pl.ds(0, 2 * D)], w_sems.at[0])
        c_v = pltpu.make_async_copy(wqkv_hbm.at[:, pl.ds(2 * D, D)],
                                    wqkv_s.at[:, pl.ds(2 * D, D)], w_sems.at[1])
        c_wo = pltpu.make_async_copy(wo_hbm, wo_s, w_sems.at[2])
        c_wing = pltpu.make_async_copy(win_hbm.at[:, pl.ds(D, D)],
                                       win_s.at[:, pl.ds(D, D)], w_sems.at[3])
        c_winu = pltpu.make_async_copy(win_hbm.at[:, pl.ds(0, D)],
                                       win_s.at[:, pl.ds(0, D)], w_sems.at[8])
        c_dwc = pltpu.make_async_copy(dwc_hbm, dwc_in, w_sems.at[4])
        c_wout = pltpu.make_async_copy(wout_hbm, wout_s, w_sems.at[5])
        c_dwm = pltpu.make_async_copy(dwm_hbm, dwm_in, w_sems.at[6])
        c_wm = pltpu.make_async_copy(wm_hbm, wm_s, w_sems.at[7])

        def ordered_start(cps):
            def body(i, c):
                for k, cp in enumerate(cps):
                    pl.when(i == k)(cp.start)
                return c
            lax.fori_loop(0, len(cps), body, 0)

        def tie(val, tok):
            if tok is None:
                return val
            true1 = one_s[0:1, :] != 0
            if val.dtype != f32:
                tok = lax.bitcast_convert_type(tok, val.dtype)
            if val.shape[1] != LANE:
                n = val.shape[1] // LANE
                return jnp.concatenate(
                    [jnp.where(true1, val[:, col(j)], tok) for j in range(n)], axis=1)
            return jnp.where(true1, val, tok)

        def toks_from(res, n):
            pts = []
            for y in res:
                for t in range(y.shape[1] // LANE):
                    for tr in range(0, y.shape[0], 8):
                        pts.append((y, t, tr))
            out = []
            for k in range(n):
                y, t, tr = pts[(k * len(pts)) // n]
                out.append(y[tr:tr + 1, col(t)])
            return out

        def conv_chunk(ref, w_ref, j, base, tok):
            acc = None
            for k in range(K):
                wk_ = tie(w_ref[k:k + 1, col(j)], tok)
                t = ref[j, pl.ds(base + k, RC), :] * wk_
                acc = t if acc is None else acc + t
            return acc

        def lnx(b, i, toks):
            for c in range(NL):
                r = rows(i, c * RL, RL)
                xb = x_s[b, r, :]
                if toks is not None:
                    xb = pltpu.bitcast(tie(pltpu.bitcast(xb, i32), toks[c]), bf16)
                xa = _ln(xb.astype(f32)).astype(bf16)
                for j in range(ND):
                    xa_s[j, r, :] = xa[:, col(j)]

        def lng(i, toks):
            for c in range(NL):
                r = rows(i, HALO + c * RL, RL, 8)
                g = jnp.concatenate([tie(g_s[j, r, :], toks[c]) for j in range(ND)], axis=1)
                g = _ln(g)
                for j in range(ND):
                    g_s[j, r, :] = g[:, col(j)]

        def proj_g(i):
            xa = cat(xa_s, rows(i))
            res = []
            for j in range(ND):
                y = jnp.dot(xa, win_s[:, D + j * LANE:D + (j + 1) * LANE],
                            preferred_element_type=f32)
                g_s[j, rows(i, HALO, TQ, 8), :] = _gelu(y)
                res.append(y)
            return res

        def proj_u(i):
            xa = cat(xa_s, rows(i))
            res = []
            for j in range(ND):
                y = jnp.dot(xa, win_s[:, col(j)], preferred_element_type=f32)
                u_s[j, rows(i), :] = _gelu(y)
                res.append(y)
            return res

        def proj_v(i):
            xa = cat(xa_s, rows(i))
            res = []
            for j in range(ND):
                y = jnp.dot(xa, wvo_s[j], preferred_element_type=f32)
                v_s[j, rows(i), :] = y.astype(bf16)
                res.append(y)
            return res

        def proj_q(i):
            xa = cat(xa_s, rows(i))
            res = []
            for j in range(ND):
                y = jnp.dot(xa, wqk_s[j], preferred_element_type=f32)
                q_s[j, rows(i), :] = y.astype(bf16)
                res.append(y)
            return res

        def prep_qk():
            wqk = lax.dot_general(wqkv_s[:, 0:D], wqkv_s[:, D:2 * D], NT,
                                  preferred_element_type=f32)
            for j in range(ND):
                wqk_s[j] = (wqk[:, col(j)] * qscale).astype(bf16)
            return wqk

        def prep_vo():
            wvo = jnp.dot(wqkv_s[:, 2 * D:3 * D], wo_s[...], preferred_element_type=f32)
            for j in range(ND):
                wvo_s[j] = wvo[:, col(j)].astype(bf16)
            return wvo

        def zcalc(i, toks):
            n = 0
            for j in range(ND):
                for r0 in range(0, TQ, RC):
                    gc = conv_chunk(g_s, dwc_s, j, i * TQ + (HALO - pad) + r0, toks[n])
                    n += 1
                    u = u_s[j, rows(i, r0, RC), :]
                    z_s[j, rows(i, r0, RC), :] = (u * gc).astype(bf16)

        def loc(i):
            z = cat(z_s, rows(i))
            res = []
            for j in range(ND):
                y = jnp.dot(z, wout_s[:, col(j)], preferred_element_type=f32)
                m_s[ND + j, rows(i, HALO, TQ, 8), :] = y
                res.append(y)
            return res

        def qk(qi, c):
            q = cat(q_s, rows(qi))
            if c == NC - 1:
                k = cat(xa_s, pl.ds(c * TK, LASTW))
                s0 = lax.dot_general(q, k, NT, preferred_element_type=f32)
                st = lax.dot_general(cat(xa_s, pl.ds(KF, REM)), cat(q_s, rows(qi, 0, QP)), NT,
                                     preferred_element_type=f32)
                st = jnp.concatenate([st, jnp.full((LANE - REM, QP), -jnp.inf, f32)], axis=0)
                s = jnp.concatenate([s0, st.T[:TQ, :]], axis=1)
            else:
                k = cat(xa_s, pl.ds(c * TK, TK))
                s = lax.dot_general(q, k, NT, preferred_element_type=f32)
            s_s[c] = s
            mx = _fold(s, jnp.maximum)
            if c == corder[0]:
                mrun[...] = mx
            else:
                mrun[...] = jnp.maximum(mrun[...], mx)
            return s

        def fin1():
            m = jnp.max(mrun[...], axis=1, keepdims=True)
            mfin[...] = jnp.broadcast_to(m, (TQ, LANE))

        def ex(c, toks):
            ps = []
            step = TQ if toks is None else RE
            for n, r0 in enumerate(range(0, TQ, step)):
                m = mfin[r0:r0 + step, :]
                if toks is not None:
                    m = tie(m, toks[n])
                mt = jnp.concatenate([m] * NKT, axis=1)
                p = jnp.exp2(s_s[c, r0:r0 + step, :] - mt)
                ls = _fold(p, jnp.add)
                if c == corder[0]:
                    l_s[r0:r0 + step, :] = ls
                else:
                    l_s[r0:r0 + step, :] += ls
                if c == NC - 1:
                    prem_s[r0:r0 + step, :] = p[:, LASTW:]
                    p = p[:, :LASTW]
                ps.append(p)
            return jnp.concatenate(ps, axis=0).astype(bf16)

        def pv(p, c):
            r = jnp.dot(p, cat(v_s, pl.ds(c * TK, p.shape[1])), preferred_element_type=f32)
            if c == corder[0]:
                acc_s[...] = r
            elif c != corder[-1]:
                acc_s[...] += r
            return r

        def pvrem(toks):
            for n, r0 in enumerate(range(0, TQ, RR)):
                pc = tie(prem_s[r0:r0 + RR, :], toks[n])
                accs = [None] * ND
                for k in range(REM):
                    pb = jnp.broadcast_to(pc[:, k:k + 1], (RR, LANE))
                    for j in range(ND):
                        t = pb * vrem_s[k:k + 1, col(j)]
                        accs[j] = t if accs[j] is None else accs[j] + t
                for j in range(ND):
                    orem_s[r0:r0 + RR, col(j)] = accs[j]

        def fin2(qi, r_last):
            l = jnp.sum(l_s[...], axis=1, keepdims=True)
            o = ((acc_s[...] + orem_s[...]) + r_last) * (1.0 / l)
            for j in range(ND):
                m_s[j, rows(qi, HALO, TQ, 8), :] = o[:, col(j)]

        def b_body(qi, carry):
            res = []
            prev = None
            for c in corder:
                p = ex(c, None if prev is None else toks_from(prev, NE))
                res.append(qk(qi + 1, c))
                r = pv(p, c)
                prev = [r[:, 0:D - LANE]]
            pvrem(toks_from(res[RPOS + 1:-1], TQ // RR))
            fin1()
            fin2(qi, r)
            return carry

        def mcalc(i, toks):
            n = 0
            for j in range(2 * ND):
                for r0 in range(0, TQ, RC):
                    mm_s[(i % 2) * 2 * ND + j, r0:r0 + RC, :] = conv_chunk(
                        m_s, dwm_s, j, i * TQ + (HALO - pad) + r0, toks[n]).astype(bf16)
                    n += 1

        def merge(b, i, stream_out):
            a = cat(mm_s, slice(None), (i % 2) * 2 * ND, (i % 2 + 1) * 2 * ND)
            res = []
            for n in range(ND):
                y = jnp.dot(a, wm_s[:, col(n)], preferred_element_type=f32)
                xr = x_s[b, rows(i), col(n)].astype(f32)
                x_s[b, rows(i), col(n)] = (xr + y).astype(bf16)
                if stream_out:
                    out_col_copy(b, i, n).start()
                res.append(y)
            return res

        ordered_start([x_copy(0, 0), c_wing, c_winu, c_qk, c_v, c_wo, x_copy(0, 1)])
        one_s[...] = jnp.ones((8, LANE), i32)
        for j in range(ND):
            xa_s[j, T:TP, :] = jnp.zeros((TP - T, LANE), bf16)
            v_s[j, T:TP, :] = jnp.zeros((TP - T, LANE), bf16)
            q_s[j, T:T - TQ + QP, :] = jnp.zeros((QP - TQ, LANE), bf16)
            g_s[j, 0:HALO, :] = jnp.zeros((HALO, LANE), f32)
            g_s[j, HALO + T:HALO + T + HALO, :] = jnp.zeros((HALO, LANE), f32)
        for j in range(2 * ND):
            m_s[j, 0:HALO, :] = jnp.zeros((HALO, LANE), f32)
            m_s[j, HALO + T:HALO + T + HALO, :] = jnp.zeros((HALO, LANE), f32)
        ordered_start([x_copy(0, 2), c_dwc, c_wout] + [x_copy(0, i) for i in range(3, NQ)])

        x_copy(0, 0).wait()
        lnx(0, 0, None)
        c_wing.wait()
        proj_g(0)
        c_winu.wait()
        lng(0, toks_from(proj_u(0), NL))
        c_qk.wait()
        prep_qk()
        proj_q(0)
        c_v.wait()
        c_wo.wait()
        x_copy(0, 1).wait()
        rv = prep_vo()
        rv2 = proj_v(0)
        lnx(0, 1, toks_from([rv] + rv2[0:ND - 1], NL))

        for b in range(B):
            if b > 0:
                for i in range(1, NQ):
                    x_copy(b, i).wait()
            for i in range(1 if b == 0 else 0, NQ):
                if b == 0 and i == 1:
                    c_dwc.wait()
                    c_wout.wait()
                    for t in range(2, 5):
                        x_copy(0, t).wait()
                    dwc_s[...] = dwc_in[...].astype(f32)
                if b == 0 and i == 4:
                    for t in range(5, NQ):
                        x_copy(0, t).wait()
                res = proj_g(i) + proj_u(i) + proj_v(i) + proj_q(i)
                if i >= 2:
                    loc(i - 2)
                if i + 1 < NQ:
                    lnx(b, i + 1, toks_from(res[0:2 * ND], NL))
                lng(i, toks_from(res[ND + 1:3 * ND], NL))
                if i >= 1:
                    zcalc(i - 1, toks_from(res[2 * ND:4 * ND], NZ))
            r8 = loc(NQ - 2)
            res = [qk(0, c) for c in corder[:NC // 2]]
            zcalc(NQ - 1, toks_from(r8 + res[0:1], NZ))
            res = [qk(0, c) for c in corder[NC // 2:]]
            fin1()
            vrem_s[...] = cat(v_s, pl.ds(KF, REM)).astype(f32)
            if b == 0:
                c_dwm.start()
                c_wm.start()
            if b + 1 < B:
                for i in range(NQ):
                    x_copy(b + 1, i).start()

            lax.fori_loop(0, NQ - 1, b_body, 0)
            if b == 0:
                c_dwm.wait()
                row = lax.broadcasted_iota(i32, (K, 2 * D), 0)
                dwm_s[...] = dwm_in[...].astype(f32) + jnp.where(row == pad, 1.0, 0.0)

            res = []
            prev = loc(NQ - 1)[0:ND - 1]
            for c in corder:
                r = pv(ex(c, toks_from(prev, NE)), c)
                res.append(r)
                prev = [r[:, 0:D - LANE]]
            pvrem(toks_from(res[RPOS + 1:-1], TQ // RR))
            mcalc(0, toks_from(res[1:], 2 * NZ))
            fin2(NQ - 1, r)
            if b == 0:
                c_wm.wait()
            else:
                for i in range(NQ):
                    out_copy(b - 1, i).wait()
            if b + 1 < B:
                x_copy(b + 1, 0).wait()

            for i in range(NQ):
                res = merge(b, i, b == B - 1 and i == NQ - 1)
                if i + 1 < NQ:
                    mcalc(i + 1, toks_from(res, 2 * NZ))
                if i == NQ - 1 and b + 1 < B:
                    lnx(b + 1, 0, toks_from(res[0:ND - 1], NL))
                if b == B - 1 and i in out_starts:
                    done = [o for o in out_starts if o < i]
                    for t in range(done[-1] + 1 if done else 0, i + 1):
                        out_copy(b, t).start()
            if b < B - 1:
                for t in range(NQ):
                    out_copy(b, t).start()

        for i in range(NQ - 1):
            out_copy(B - 1, i).wait()
        for n in range(ND):
            out_col_copy(B - 1, NQ - 1, n).wait()

    any_spec = pl.BlockSpec(memory_space=pl.ANY)
    return pl.pallas_call(
        kernel,
        out_shape=jax.ShapeDtypeStruct((B, T, D), x.dtype),
        in_specs=[any_spec] * 8,
        out_specs=any_spec,
        scratch_shapes=[
            pltpu.VMEM((B, T, D), bf16),
            pltpu.VMEM((D, 3 * D), bf16),
            pltpu.VMEM((D, D), bf16),
            pltpu.VMEM((D, 2 * D), bf16),
            pltpu.VMEM((D, D), bf16),
            pltpu.VMEM((2 * D, D), bf16),
            pltpu.VMEM((K, D), bf16),
            pltpu.VMEM((K, 2 * D), bf16),
            pltpu.VMEM((ND, D, LANE), bf16),
            pltpu.VMEM((ND, D, LANE), bf16),
            pltpu.VMEM((K, D), f32),
            pltpu.VMEM((K, 2 * D), f32),
            pltpu.VMEM((8, LANE), i32),
            pltpu.VMEM((ND, TP, LANE), bf16),
            pltpu.VMEM((ND, T - TQ + QP, LANE), bf16),
            pltpu.VMEM((ND, TP, LANE), bf16),
            pltpu.VMEM((ND, T, LANE), f32),
            pltpu.VMEM((ND, T + 2 * HALO, LANE), f32),
            pltpu.VMEM((2 * ND, T + 2 * HALO, LANE), f32),
            pltpu.VMEM((ND, T, LANE), bf16),
            pltpu.VMEM((4 * ND, TQ, LANE), bf16),
            pltpu.VMEM((NC, TQ, TK), f32),
            pltpu.VMEM((TQ, LANE), f32),
            pltpu.VMEM((TQ, LANE), f32),
            pltpu.VMEM((TQ, LANE), f32),
            pltpu.VMEM((TQ, D), f32),
            pltpu.VMEM((TQ, LANE), f32),
            pltpu.VMEM((REM, D), f32),
            pltpu.VMEM((TQ, D), f32),
            pltpu.SemaphoreType.DMA((9 + ND,)),
            pltpu.SemaphoreType.DMA((B * NQ,)),
        ],
        compiler_params=pltpu.CompilerParams(vmem_limit_bytes=120 * 1024 * 1024),
    )(x, w_qkv, w_att_out, w_mlp_in, dw_csgu, w_mlp_out, dw_merge, w_merge)
```
